```python
import os as _os
_os.environ.setdefault("JAX_PLATFORMS", "cpu")
import jax
import jax.numpy as jnp

def _softmax(x, axis=-1):
    return jax.nn.softmax(x, axis=axis)
def _gelu(x):
    return jax.nn.gelu(x, approximate=True)
def _silu(x):
    return jax.nn.silu(x)
def _sigmoid(x):
    return jax.nn.sigmoid(x)
def _layernorm(x, axis=-1, eps=1e-5):
    m = jnp.mean(x, axis=axis, keepdims=True)
    v = jnp.var(x, axis=axis, keepdims=True)
    return (x - m) / jnp.sqrt(v + eps)
def _scatter_add(tgt, idx, src, axis=0):
    return tgt.at[idx].add(src)
def _segment_sum(src, seg, n):
    return jax.ops.segment_sum(src, seg, n)
class _Rng:
    def __init__(self, key):
        self._k = key
    def _next(self):
        self._k, sub = jax.random.split(self._k)
        return sub
    def normal(self, shape):
        return jax.random.normal(self._next(), shape, dtype=jnp.bfloat16)
    def randint(self, lo, hi, shape):
        return jax.random.randint(self._next(), shape, lo, hi, dtype=jnp.int32)
    def uniform(self, shape, lo=0.0, hi=1.0):
        return jax.random.uniform(self._next(), shape, jnp.bfloat16, lo, hi)
    def permutation(self, n):
        return jax.random.permutation(self._next(), n)


kernel_name = 'gated_mix__sliding_block__dense_activation_silu__prompt'

def setup_inputs():
    _rng = _Rng(jax.random.key(int.from_bytes(__import__("os").urandom(4), "little")))
    _w = (lambda a: (lambda t: t.astype(jnp.bfloat16) if jnp.issubdtype(t.dtype, jnp.floating) else t)(jnp.asarray(a)))
    def _A_setup():
        B, S, D = 1, 2048, 640
        return {
            "x": _w((lambda *s: _rng.normal(s) * 0.05)(B, S, D)),
            "wqkv": _w((lambda *s: _rng.normal(s) * 0.4)(D, 3 * D)),
            "wo": _w((lambda *s: _rng.normal(s) * 0.05)(D, D)),
        }
    _A_in = _A_setup()

    def _B_setup():
        B, S, D, F = 1, 2048, 640, 1536
        return {
            "x": _w((lambda *s: _rng.normal(s) * 0.05)(B, S, D)),
            "w1": _w((lambda *s: _rng.normal(s) * 1.6)(D, F) * (D ** -0.5)),
            "w2": _w((lambda *s: _rng.normal(s) * 1.6)(F, D) * (F ** -0.5)),
        }
    _B_in = _B_setup()

    return {
        "A_x": _A_in["x"],
        "A_wqkv": _A_in["wqkv"],
        "A_wo": _A_in["wo"],
        "B_x": _B_in["x"],
        "B_w1": _B_in["w1"],
        "B_w2": _B_in["w2"],
        "gate_w": _w((lambda *s: _rng.normal(s) * 0.05)(640) * 16.0),
    }

def reference(A_x, A_wqkv, A_wo, B_x, B_w1, B_w2, gate_w):
    def _A_ref(x, wqkv, wo):
        B, S, D = x.shape
        H = 32; Dh = D // H; W = 256
        qkv = (lambda x, *d: x.transpose(*d))((x @ wqkv).reshape(B, S, 3, H, Dh), 2, 0, 3, 1, 4)
        q, k, v = qkv[0], qkv[1], qkv[2]
        scores = jnp.einsum("bhqd,bhkd->bhqk", q, k) * (Dh ** -0.5)
        idx = jnp.arange(S)
        mask = (idx[:, None] - idx[None, :] >= 0) & (idx[:, None] - idx[None, :] < W)
        scores = jnp.where(mask[None, None], scores, -1e9)
        p = _softmax(scores, axis=-1)
        o = jnp.einsum("bhqk,bhkd->bhqd", p, v)
        return (lambda x, *d: x.transpose(*d))(o, 0, 2, 1, 3).reshape(B, S, D) @ wo

    def _B_ref(x, w1, w2):
        h = jnp.einsum("bsd,df->bsf", x, w1)
        h = _silu(h)
        out = jnp.einsum("bsf,fd->bsd", h, w2)
        return out

    x = A_x
    g = _sigmoid((x * gate_w).sum(-1, keepdims=True))
    a = _A_ref(x, A_wqkv, A_wo)
    b = _B_ref(x, B_w1, B_w2)
    return g * a + (1 - g) * b
```

```python
import functools
import numpy as np
import jax
import jax.numpy as jnp
from jax import lax
import jax.experimental.pallas as pl
import jax.experimental.pallas.tpu as pltpu

S, D, H, DH, F, W = 2048, 640, 32, 20, 1536, 256
NG = 8
QB = 128
LOG2E = 1.4426950408889634
NEG = -1e30

def _slabs(t):
    nat = [t[:, 128 * s:128 * (s + 1)] for s in range(5)]
    lane = lax.broadcasted_iota(jnp.int32, nat[0].shape, 1)
    out = []
    for g in range(NG):
        lo = 80 * g
        s0, off = lo // 128, lo % 128
        if off + 80 <= 128:
            out.append(nat[s0])
        else:
            out.append(jnp.where(lane >= off, nat[s0], nat[s0 + 1]))
    return out

def _kernel(x_ref, wqkv_ref, wo_ref, w1_ref, w2_ref, gw_ref, out_ref,
            k_scr, vT_scr, wvT_scr, sA, sB, b1_scr, b3_scr, pA, pB, *, T, PIPE, OPQ):
    i = pl.program_id(0)
    f32, bf16, i32 = jnp.float32, jnp.bfloat16, jnp.int32
    s_l = [sA, sB]; p_l = [pA, pB]
    z = jnp.minimum(i, 0) if OPQ else 0

    @pl.when(i == 0)
    def _():
        wvT_scr[...] = wqkv_ref[:, 2 * D:3 * D].astype(f32).T.astype(bf16)
        k_scr[:, 0:W, :] = jnp.zeros((NG, W, 128), bf16)
        vT_scr[:, 0:W] = jnp.zeros((H * 32, W), bf16)

    x = x_ref[...]
    qk = jnp.dot(x, wqkv_ref[:, 0:2 * D], preferred_element_type=f32)
    q = qk[:, :D] * (DH ** -0.5 * LOG2E)
    k = qk[:, D:]
    qs = [pltpu.bitcast(s.astype(bf16), i32) for s in _slabs(q)]
    ks = [s.astype(bf16) for s in _slabs(k)]
    base = pl.multiple_of(i * T, T)
    for g in range(NG):
        k_scr[g, pl.ds(base + W, T), :] = ks[g]
    vT = lax.dot_general(wvT_scr[...], x, (((1,), (1,)), ((), ())), preferred_element_type=f32)
    rowi = lax.broadcasted_iota(i32, (32, T), 0)
    for hd in range(H):
        g, hh = hd // 4, hd % 4
        hm = (rowi >= 4 * hh) & (rowi < 4 * hh + DH)
        r0 = 80 * g + 16 * hh
        vT_scr[32 * hd:32 * hd + 32, pl.ds(base + W, T)] = jnp.where(hm, vT[r0:r0 + 32], 1.0).astype(bf16)

    h = jnp.dot(x, w1_ref[...], preferred_element_type=f32)
    h = (h * jax.nn.sigmoid(h)).astype(bf16)
    b = jnp.dot(h, w2_ref[...], preferred_element_type=f32)
    gl = jnp.sum(x.astype(f32) * gw_ref[...].astype(f32), axis=1, keepdims=True)
    gate = jax.nn.sigmoid(gl)

    r = lax.broadcasted_iota(i32, (QB, QB), 0)
    c = lax.broadcasted_iota(i32, (QB, QB), 1)
    lane64 = lax.broadcasted_iota(i32, (QB // 2, 128), 1)
    row8 = lax.broadcasted_iota(i32, (8, QB), 0)
    b3_scr[...] = jnp.where(r <= c, 0.0, NEG).astype(f32)
    for jj in range(T // QB):
        q0 = base + jj * QB
        b1_scr[...] = jnp.where((r > c) & (q0 >= 256), 0.0, NEG).astype(f32)
        bias2 = jnp.where(q0 >= 128, 0.0, NEG).astype(f32)

        def qmask(g):
            qslab = qs[g][jj * QB // 2:(jj + 1) * QB // 2]
            qm = []
            for hh in range(4):
                hd = 4 * g + hh
                lm = ((lane64 - 20 * hd) & 127) < DH
                qm.append(jnp.where(lm, qslab, 0))
            return pltpu.bitcast(jnp.concatenate(qm, axis=0), bf16)

        def qk_t(g, slot, t, qm, mrun):
            kw = k_scr[g, pl.ds(q0 + t * QB, QB), :]
            sT = lax.dot_general(kw, qm, (((1,), (1,)), ((), ())), preferred_element_type=f32)
            out = []
            for hh in range(4):
                cs = slice(hh * QB, (hh + 1) * QB)
                if t == 0:
                    s = sT[:, cs] + b1_scr[...]
                elif t == 1:
                    s = sT[:, cs] + bias2
                else:
                    s = sT[:, cs] + b3_scr[...]
                s_l[slot][z, 3 * hh + t] = s
                mm = s[0:8]
                for r8 in range(1, 16):
                    mm = jnp.maximum(mm, s[8 * r8:8 * r8 + 8])
                out.append(mm if mrun is None else jnp.maximum(mrun[hh], mm))
            return out

        def exp_t(g, slot, t, ms):
            for hh in range(4):
                p_l[slot][z, 3 * hh + t] = jnp.exp2(s_l[slot][z, 3 * hh + t] - ms[hh]).astype(bf16)

        def pv_all(g, slot):
            acc = []
            for hh in range(4):
                hd = 4 * g + hh
                o = None
                for t in range(3):
                    vw = vT_scr[32 * hd:32 * hd + 32, pl.ds(q0 + t * QB, QB)]
                    d = jnp.dot(vw, p_l[slot][z, 3 * hh + t], preferred_element_type=f32)
                    o = d if o is None else o + d
                acc.append(o)
            return acc

        def pv_t(g, slot, t, ms, acc):
            out = []
            for hh in range(4):
                hd = 4 * g + hh
                p = jnp.exp2(s_l[slot][z, 3 * hh + t] - ms[hh]).astype(bf16)
                vw = vT_scr[32 * hd:32 * hd + 32, pl.ds(q0 + t * QB, QB)]
                d = jnp.dot(vw, p, preferred_element_type=f32)
                out.append(d if acc is None else acc[hh] + d)
            return out

        def finish(acc):
            os_ = []
            for hh in range(4):
                o = acc[hh]
                lrow = 31 if hh < 3 else 0
                l = o[lrow:lrow + 1, :]
                os_.append(o * (1.0 / l))
            o0, o1, o2, o3 = os_
            return [o0[0:16], jnp.where(row8 < 4, o0[16:24], o1[0:8]), o1[8:24], o2[8:24],
                    jnp.where(row8 < 4, o2[24:32], o3[8:16]), o3[16:32]]

        def fin_max(mrun):
            return [jnp.max(m, axis=0, keepdims=True) for m in mrun]

        groups = []
        qm = qmask(0)
        mrun = None
        for t in range(3):
            mrun = qk_t(0, 0, t, qm, mrun)
        for g in range(NG):
            ms = fin_max(mrun)
            mrun = None
            sl_, sn = g % 2, (g + 1) % 2
            if g + 1 < NG:
                qm = qmask(g + 1)
            if PIPE in (1, 2, 3):
                if PIPE == 1:
                    for t in range(3):
                        if g + 1 < NG:
                            mrun = qk_t(g + 1, sn, t, qm, mrun)
                        exp_t(g, sl_, t, ms)
                elif PIPE == 2:
                    for t in range(3):
                        exp_t(g, sl_, t, ms)
                        if g + 1 < NG:
                            mrun = qk_t(g + 1, sn, t, qm, mrun)
                else:
                    for t in range(3):
                        exp_t(g, sl_, t, ms)
                    for t in range(3):
                        if g + 1 < NG:
                            mrun = qk_t(g + 1, sn, t, qm, mrun)
                groups += finish(pv_all(g, sl_))
            else:
                acc = None
                for t in range(3):
                    if PIPE == 4 and g + 1 < NG:
                        mrun = qk_t(g + 1, sn, t, qm, mrun)
                    acc = pv_t(g, sl_, t, ms, acc)
                    if PIPE == 5 and g + 1 < NG:
                        mrun = qk_t(g + 1, sn, t, qm, mrun)
                groups += finish(acc)
        oT = jnp.concatenate(groups, axis=0)
        o = oT.T.astype(bf16)
        a = jnp.dot(o, wo_ref[...], preferred_element_type=f32)
        sl = slice(jj * QB, (jj + 1) * QB)
        gj = gate[sl]
        out_ref[sl, :] = (gj * a + (1.0 - gj) * b[sl]).astype(out_ref.dtype)

@functools.partial(jax.jit, static_argnames=("T", "PIPE", "OPQ"))
def pallas_gated_mix__sliding_block__dense_activation_silu__prompt_kernel(A_x, A_wqkv, A_wo, B_x, B_w1, B_w2, gate_w, T=128, PIPE=4, OPQ=True):
    x = A_x.reshape(S, D)
    gw = gate_w.reshape(1, D)
    const = lambda i: (0, 0)
    out = pl.pallas_call(
        functools.partial(_kernel, T=T, PIPE=PIPE, OPQ=OPQ),
        grid=(S // T,),
        in_specs=[pl.BlockSpec((T, D), lambda i: (i, 0)),
                  pl.BlockSpec((D, 3 * D), const), pl.BlockSpec((D, D), const),
                  pl.BlockSpec((D, F), const), pl.BlockSpec((F, D), const), pl.BlockSpec((1, D), const)],
        out_specs=pl.BlockSpec((T, D), lambda i: (i, 0)),
        out_shape=jax.ShapeDtypeStruct((S, D), jnp.bfloat16),
        scratch_shapes=[pltpu.VMEM((NG, W + S, 128), jnp.bfloat16), pltpu.VMEM((H * 32, W + S), jnp.bfloat16),
                        pltpu.VMEM((D, D), jnp.bfloat16),
                        pltpu.VMEM((1, 12, QB, QB), jnp.float32), pltpu.VMEM((1, 12, QB, QB), jnp.float32),
                        pltpu.VMEM((QB, QB), jnp.float32), pltpu.VMEM((QB, QB), jnp.float32),
                        pltpu.VMEM((1, 12, QB, QB), jnp.bfloat16), pltpu.VMEM((1, 12, QB, QB), jnp.bfloat16)],
        compiler_params=pltpu.CompilerParams(dimension_semantics=("arbitrary",), vmem_limit_bytes=100 * 2**20),
    )(x, A_wqkv, A_wo, B_w1, B_w2, gw)
    return out.reshape(1, S, D)
```

```python
import functools
import numpy as np
import jax
import jax.numpy as jnp
from jax import lax
import jax.experimental.pallas as pl
import jax.experimental.pallas.tpu as pltpu

S, D, H, DH, F, W = 2048, 640, 32, 20, 1536, 256
NG = 8
QB = 128
LOG2E = 1.4426950408889634
NEG = -1e30
f32, bf16, i32 = jnp.float32, jnp.bfloat16, jnp.int32
NT_DIMS = (((1,), (1,)), ((), ()))

def _slabs(t):
    nat = [t[:, 128 * s:128 * (s + 1)] for s in range(5)]
    lane = lax.broadcasted_iota(i32, nat[0].shape, 1)
    out = []
    for g in range(NG):
        lo = 80 * g
        s0, off = lo // 128, lo % 128
        if off + 80 <= 128:
            out.append(nat[s0])
        else:
            out.append(jnp.where(lane >= off, nat[s0], nat[s0 + 1]))
    return out

def _kernel(x_hbm, wqkv_hbm, wo_hbm, w1_hbm, w2_hbm, gw_ref, out_hbm,
            x_v, wqkv_v, wo_v, w1_v, w2_v, wT_v, q_scr, k_scr, vT_scr, sA, sB, ba_scr, bm_scr, bc_scr, o_scr, h_scr, b_scr, out_v,
            sem_x, sem_x0, sem_w, sem_o, *, TP, T, F1C, F1R, TAILJ, SPREAD):
    NP = S // TP
    T0 = TP // 2
    def xcopy(j):
        return pltpu.make_async_copy(x_hbm.at[pl.ds(j * TP, TP), :], x_v.at[pl.ds(j * TP, TP), :], sem_x.at[j])
    def xcopy0(hf):
        return pltpu.make_async_copy(x_hbm.at[pl.ds(hf * T0, T0), :], x_v.at[pl.ds(hf * T0, T0), :], sem_x0.at[hf])
    wcopies = [
        pltpu.make_async_copy(wqkv_hbm.at[:, pl.ds(0, D)], wqkv_v.at[:, pl.ds(0, D)], sem_w.at[0]),
        pltpu.make_async_copy(wqkv_hbm.at[:, pl.ds(D, D)], wqkv_v.at[:, pl.ds(D, D)], sem_w.at[1]),
        pltpu.make_async_copy(wqkv_hbm.at[:, pl.ds(2 * D, D)], wqkv_v.at[:, pl.ds(2 * D, D)], sem_w.at[2]),
        pltpu.make_async_copy(w1_hbm, w1_v, sem_w.at[3]),
        pltpu.make_async_copy(w2_hbm, w2_v, sem_w.at[4]),
        pltpu.make_async_copy(wo_hbm, wo_v, sem_w.at[5]),
    ]
    xcopy0(0).start()
    wcopies[1].start()

    k_scr[:, 0:W // 2, :] = jnp.zeros((NG, W // 2, 128), i32)
    vT_scr[:, 0:W] = jnp.zeros((H * 32, W), bf16)
    r = lax.broadcasted_iota(i32, (QB, QB), 0)
    c = lax.broadcasted_iota(i32, (QB, QB), 1)
    r64 = lax.broadcasted_iota(i32, (64, QB), 0)
    c64 = lax.broadcasted_iota(i32, (64, QB), 1)
    bc_scr[...] = jnp.where(r64 <= c64, 0.0, NEG).astype(f32)

    def proj_k(base, hbase, n):
        x = x_v[pl.ds(base, n), :]
        k = jnp.dot(x, wqkv_v[:, D:2 * D], preferred_element_type=f32)
        for g, s in enumerate(_slabs(k)):
            k_scr[g, pl.ds(hbase + W // 2, n // 2), :] = pltpu.bitcast(s.astype(bf16), i32)

    def proj_q(base, n):
        x = x_v[pl.ds(base, n), :]
        qT = lax.dot_general(wT_v[0:D, :], x, NT_DIMS, preferred_element_type=f32) * (DH ** -0.5 * LOG2E)
        q_scr[:, pl.ds(base, n)] = pltpu.bitcast(qT.astype(bf16), i32)

    def proj_v(base, n):
        x = x_v[pl.ds(base, n), :]
        vT = lax.dot_general(wT_v[D:2 * D, :], x, NT_DIMS, preferred_element_type=f32)
        rowi = lax.broadcasted_iota(i32, (32, n), 0)
        for hd in range(H):
            g, hh = hd // 4, hd % 4
            hm = (rowi >= 4 * hh) & (rowi < 4 * hh + DH)
            r0 = 80 * g + 16 * hh
            vT_scr[32 * hd:32 * hd + 32, pl.ds(base + W, n)] = jnp.where(hm, vT[r0:r0 + 32], 1.0).astype(bf16)

    xcopy0(0).wait()
    xcopy0(1).start()
    wcopies[0].start()
    wcopies[1].wait()
    wcopies[2].start()
    proj_k(0, 0, T0)
    xcopy0(1).wait()
    for j in range(1, NP):
        xcopy(j).start()
    for cp in wcopies[3:]:
        cp.start()
    proj_k(T0, T0 // 2, T0)
    wcopies[0].wait()
    wT_v[0:D, :] = wqkv_v[:, 0:D].astype(f32).T.astype(bf16)
    proj_q(0, TP)
    wcopies[2].wait()
    wT_v[D:2 * D, :] = wqkv_v[:, 2 * D:3 * D].astype(f32).T.astype(bf16)
    proj_v(0, TP)
    def proj_loop(j, carry):
        xcopy(j).wait()
        base = pl.multiple_of(j * TP, TP)
        proj_k(base, pl.multiple_of(j * (TP // 2), TP // 2), TP)
        proj_q(base, TP)
        proj_v(base, TP)
        return carry
    lax.fori_loop(1, NP, proj_loop, 0)

    for cp in wcopies[3:]:
        cp.wait()

    s_l = [sA, sB]
    NQ = T // QB
    lane64 = lax.broadcasted_iota(i32, (QB // 2, 128), 1)
    lane32 = lax.broadcasted_iota(i32, (32, 128), 1)
    row8 = lax.broadcasted_iota(i32, (8, QB), 0)
    col8 = lax.broadcasted_iota(i32, (8, QB), 1)

    def ocopy(i):
        return pltpu.make_async_copy(out_v.at[pl.ds(i * T, T), :], out_hbm.at[pl.ds(i * T, T), :], sem_o.at[i])

    def body(i, carry):
        base = pl.multiple_of(i * T, T)
        z = jnp.minimum(i, 0)
        x = x_v[pl.ds(base, T), :]
        biases = []
        for jj in range(NQ):
            q0 = base + jj * QB
            ok = q0 >= 256
            ba_scr[jj] = jnp.where((r64 + 64 > c64) & ok, 0.0, NEG).astype(f32)
            bm_scr[jj] = jnp.where(c64 < 64, jnp.where((r64 > c64) & ok, 0.0, NEG), jnp.where(r64 <= c64 - 64, 0.0, NEG)).astype(f32)
            biases.append(jnp.where(q0 >= 128, 0.0, NEG).astype(f32))

        def krows(g, jj, r0, n):
            st = pl.multiple_of(base // 2 + (jj * QB + r0) // 2, 32)
            return k_scr[g, pl.ds(st, n // 2), :]

        def qmask(u):
            jj, g = u // NG, u % NG
            qv = q_scr[40 * g:40 * g + 40, pl.ds(pl.multiple_of(base + jj * QB, QB), QB)]
            zero = jnp.zeros((8, QB), i32)
            qm, qc = [], []
            for hh in range(4):
                blocks = [zero] * 8
                for v in range(5):
                    lo, hi = max(10 * hh, 8 * v), min(10 * hh + 10, 8 * v + 8)
                    if lo >= hi:
                        continue
                    blk = qv[8 * v:8 * v + 8]
                    if hi - lo < 8:
                        blk = jnp.where((row8 >= lo - 8 * v) & (row8 < hi - 8 * v), blk, 0)
                    blocks[(5 * g + v) % 8] = blk
                qm.append(jnp.concatenate(blocks, axis=0))
                cb = []
                for b in range(8):
                    a_, b_ = blocks[b], blocks[(b + 4) % 8]
                    if a_ is zero and b_ is zero:
                        cb.append(zero)
                    elif b_ is zero:
                        cb.append(jnp.where(col8 < 64, a_, 0))
                    elif a_ is zero:
                        cb.append(jnp.where(col8 >= 64, b_, 0))
                    else:
                        cb.append(jnp.where(col8 < 64, a_, b_))
                qc.append(jnp.concatenate(cb, axis=0))
            return (pltpu.bitcast(jnp.concatenate(qm, axis=1), bf16),
                    pltpu.bitcast(jnp.concatenate(qc, axis=1), bf16))

        def vmax8(s):
            mm = s[0:8]
            for r8 in range(1, s.shape[0] // 8):
                mm = jnp.maximum(mm, s[8 * r8:8 * r8 + 8])
            return mm

        def qk_piece(u, t, qms, mrun):
            jj, g = u // NG, u % NG
            slot = u % 2
            qm, qc = qms
            out = []
            if t == 2:
                early = krows(g, jj, 0, 64)
                late = pltpu.roll(krows(g, jj, 320, 64), 64, 1)
                o = (80 * g) % 128
                sTs = []
                for pr in range(2):
                    lsel = ((lane32 - (o + 40 * pr + 64)) & 127) < 40
                    lhs = pltpu.bitcast(jnp.where(lsel, late, early), bf16)
                    sTs.append(jnp.dot(lhs, qc[:, 256 * pr:256 * pr + 256], preferred_element_type=f32))
                for hh in range(4):
                    s = sTs[hh // 2][:, (hh % 2) * QB:(hh % 2 + 1) * QB] + bm_scr[jj]
                    s_l[slot][z, hh, 256:320] = s
                    mm = vmax8(s)
                    out.append(mm if mrun is None else jnp.maximum(mrun[hh], mm))
                return out
            kw = pltpu.bitcast(krows(g, jj, 64 + 128 * t, 128), bf16)
            sT = jnp.dot(kw, qm, preferred_element_type=f32)
            for hh in range(4):
                s = sT[:, hh * QB:(hh + 1) * QB]
                if t == 0:
                    s = jnp.concatenate([s[0:64] + ba_scr[jj], s[64:128] + biases[jj]], axis=0)
                else:
                    s = jnp.concatenate([s[0:64] + biases[jj], s[64:128] + bc_scr[...]], axis=0)
                s_l[slot][z, hh, 128 * t:128 * t + 128] = s
                mm = vmax8(s)
                out.append(mm if mrun is None else jnp.maximum(mrun[hh], mm))
            return out

        cl = lax.broadcasted_iota(i32, (32, QB), 1)
        def pv_t(u, t, ms, acc):
            jj, g = u // NG, u % NG
            slot = u % 2
            out = []
            for hh in range(4):
                hd = 4 * g + hh
                ex = lambda r0, n: jnp.exp2(s_l[slot][z, hh, r0:r0 + n] - ms[hh]).astype(bf16)
                if t == 0:
                    pm = pltpu.bitcast(ex(256, 64), i32)
                    p = jnp.concatenate([jnp.where(cl < 64, pm, 0), pltpu.bitcast(ex(0, 64), i32)], axis=0)
                    p = pltpu.bitcast(p, bf16)
                elif t == 1:
                    p = ex(64, 128)
                else:
                    pm = pltpu.bitcast(ex(256, 64), i32)
                    p = jnp.concatenate([pltpu.bitcast(ex(192, 64), i32), jnp.where(cl >= 64, pm, 0)], axis=0)
                    p = pltpu.bitcast(p, bf16)
                vw = vT_scr[32 * hd:32 * hd + 32, pl.ds(pl.multiple_of(base + (jj + t) * QB, QB), QB)]
                d = jnp.dot(vw, p, preferred_element_type=f32)
                out.append(d if acc is None else acc[hh] + d)
            return out

        def finish(u, acc):
            jj, g = u // NG, u % NG
            os_ = []
            for hh in range(4):
                o = acc[hh]
                lrow = 31 if hh < 3 else 0
                l = o[lrow:lrow + 1, :]
                os_.append(o * (1.0 / l))
            o0, o1, o2, o3 = os_
            o_scr[jj, 80 * g:80 * g + 80, :] = jnp.concatenate(
                [o0[0:16], jnp.where(row8 < 4, o0[16:24], o1[0:8]), o1[8:24], o2[8:24],
                 jnp.where(row8 < 4, o2[24:32], o3[8:16]), o3[16:32]], axis=0)

        fin_max = lambda mrun: [jnp.max(m, axis=0, keepdims=True) for m in mrun]

        gl = jnp.sum(x.astype(f32) * gw_ref[...].astype(f32).reshape(1, D), axis=1, keepdims=True)
        gate = 0.5 * jnp.tanh(0.5 * gl) + 0.5
        hg = 0.5 * (1.0 - gate)

        def ffn1(r0, r1, c0, c1):
            h = jnp.dot(x[r0:r1], w1_v[:, c0:c1], preferred_element_type=f32)
            h = (h * hg[r0:r1]) * (jnp.tanh(0.5 * h) + 1.0)
            h_scr[r0:r1, c0:c1] = h.astype(bf16)

        def ffn2(n0, n1):
            b_scr[:, n0:n1] = jnp.dot(h_scr[...], w2_v[:, n0:n1], preferred_element_type=f32)
        jobs = []
        for c0 in range(0, F, F1C):
            for r0 in range(0, T, F1R):
                jobs.append(functools.partial(ffn1, r0, r0 + F1R, c0, c0 + F1C))
        jobs.append(functools.partial(ffn2, 512, D))
        NU = NQ * NG
        nj = len(jobs)
        tail_jobs = TAILJ
        spread = jobs[:nj - tail_jobs]
        per_unit = [[] for _ in range(NU)]
        for ji, jb in enumerate(spread):
            per_unit[(ji * (NU - 1)) // max(len(spread) - 1, 1) if SPREAD else NU - 1].append(jb)
        tails = jobs[nj - tail_jobs:]
        qm = qmask(0)
        mrun = None
        for t in range(3):
            mrun = qk_piece(0, t, qm, mrun)
        for u in range(NU):
            ms = fin_max(mrun)
            mrun = None
            acc = None
            if u + 1 < NU:
                qm = qmask(u + 1)
                for t in range(3):
                    mrun = qk_piece(u + 1, t, qm, mrun)
                    acc = pv_t(u, t, ms, acc)
                    if t < len(per_unit[u]):
                        per_unit[u][t]()
                for jb in per_unit[u][3:]:
                    jb()
            else:
                for jb in per_unit[u]:
                    jb()
                if len(tails) > 1:
                    tails[0]()
                for t in range(3):
                    acc = pv_t(u, t, ms, acc)
            finish(u, acc)
        for jb in tails[1 if len(tails) > 1 else 0:]:
            jb()
        accs = []
        for jj in range(NQ):
            o = (o_scr[jj].T * gate[jj * QB:(jj + 1) * QB]).astype(bf16)
            accs.append(o)
        o_all = jnp.concatenate(accs, axis=0)
        a = jnp.dot(o_all, wo_v[...], preferred_element_type=f32)
        out_v[pl.ds(base, T), 512:D] = (a[:, 512:D] + b_scr[:, 512:D]).astype(bf16)
        b0 = jnp.dot(h_scr[...], w2_v[:, 0:512], preferred_element_type=f32)
        out_v[pl.ds(base, T), 0:512] = (a[:, 0:512] + b0).astype(bf16)
        ocopy(i).start()
        return carry
    lax.fori_loop(0, S // T, body, 0)
    for i in range(S // T):
        ocopy(i).wait()

@functools.partial(jax.jit, static_argnames=("T", "TP", "F1C", "F1R", "TAILJ", "SPREAD"))
def pallas_gated_mix__sliding_block__dense_activation_silu__prompt_kernel(A_x, A_wqkv, A_wo, B_x, B_w1, B_w2, gate_w, T=256, TP=512, F1C=128, F1R=128, TAILJ=3, SPREAD=True):
    x = A_x.reshape(S, D)
    gw = gate_w
    anyspec = pl.BlockSpec(memory_space=pl.ANY)
    NQ = T // QB
    out = pl.pallas_call(
        functools.partial(_kernel, TP=TP, T=T, F1C=F1C, F1R=F1R, TAILJ=TAILJ, SPREAD=SPREAD),
        in_specs=[anyspec] * 5 + [pl.BlockSpec(memory_space=pltpu.VMEM)],
        out_specs=anyspec,
        out_shape=jax.ShapeDtypeStruct((S, D), bf16),
        scratch_shapes=[
            pltpu.VMEM((S, D), bf16), pltpu.VMEM((D, 3 * D), bf16), pltpu.VMEM((D, D), bf16),
            pltpu.VMEM((D, F), bf16), pltpu.VMEM((F, D), bf16), pltpu.VMEM((2 * D, D), bf16),
            pltpu.VMEM((D // 2, S), i32), pltpu.VMEM((NG, (W + S) // 2, 128), i32), pltpu.VMEM((H * 32, W + S), bf16),
            pltpu.VMEM((1, 4, 320, QB), f32), pltpu.VMEM((1, 4, 320, QB), f32),
            pltpu.VMEM((NQ, 64, QB), f32), pltpu.VMEM((NQ, 64, QB), f32), pltpu.VMEM((64, QB), f32),
            pltpu.VMEM((NQ, D, QB), f32), pltpu.VMEM((T, F), bf16), pltpu.VMEM((T, D), f32), pltpu.VMEM((S, D), bf16),
            pltpu.SemaphoreType.DMA((S // TP,)), pltpu.SemaphoreType.DMA((2,)), pltpu.SemaphoreType.DMA((6,)), pltpu.SemaphoreType.DMA((S // T,))],
        compiler_params=pltpu.CompilerParams(vmem_limit_bytes=100 * 2**20),
    )(x, A_wqkv, A_wo, B_w1, B_w2, gw)
    return out.reshape(1, S, D)
```

```python
import functools
import numpy as np
import jax
import jax.numpy as jnp
from jax import lax
import jax.experimental.pallas as pl
import jax.experimental.pallas.tpu as pltpu

S, D, H, DH, F, W = 2048, 640, 32, 20, 1536, 256
NG = 8
QB = 128
LOG2E = 1.4426950408889634
NEG = -1e30
f32, bf16, i32 = jnp.float32, jnp.bfloat16, jnp.int32
NT_DIMS = (((1,), (1,)), ((), ()))

def _slabs(t):
    nat = [t[:, 128 * s:128 * (s + 1)] for s in range(5)]
    lane = lax.broadcasted_iota(i32, nat[0].shape, 1)
    out = []
    for g in range(NG):
        lo = 80 * g
        s0, off = lo // 128, lo % 128
        if off + 80 <= 128:
            out.append(nat[s0])
        else:
            out.append(jnp.where(lane >= off, nat[s0], nat[s0 + 1]))
    return out

def _kernel(x_hbm, wqkv_hbm, wo_hbm, w1_hbm, w2_hbm, gw_ref, out_hbm,
            x_v, wqkv_v, wo_v, w1_v, w2_v, wT_v, q_scr, k_scr, vT_scr, sA, sB, ba_scr, bm_scr, bc_scr, pm_scr, o_scr, h_scr, b_scr, out_v,
            sem_x, sem_x0, sem_w, sem_o, *, TP, T, F1C, F1R, TAILJ, SPREAD, OP):
    NP = S // TP
    T0 = TP // 2
    def xcopy(j):
        return pltpu.make_async_copy(x_hbm.at[pl.ds(j * TP, TP), :], x_v.at[pl.ds(j * TP, TP), :], sem_x.at[j])
    def xcopy0(hf):
        return pltpu.make_async_copy(x_hbm.at[pl.ds(hf * T0, T0), :], x_v.at[pl.ds(hf * T0, T0), :], sem_x0.at[hf])
    wcopies = [
        pltpu.make_async_copy(wqkv_hbm.at[:, pl.ds(0, D)], wqkv_v.at[:, pl.ds(0, D)], sem_w.at[0]),
        pltpu.make_async_copy(wqkv_hbm.at[:, pl.ds(D, D)], wqkv_v.at[:, pl.ds(D, D)], sem_w.at[1]),
        pltpu.make_async_copy(wqkv_hbm.at[:, pl.ds(2 * D, D)], wqkv_v.at[:, pl.ds(2 * D, D)], sem_w.at[2]),
        pltpu.make_async_copy(w1_hbm, w1_v, sem_w.at[3]),
        pltpu.make_async_copy(w2_hbm, w2_v, sem_w.at[4]),
        pltpu.make_async_copy(wo_hbm, wo_v, sem_w.at[5]),
    ]
    xcopy0(0).start()
    wcopies[1].start()

    k_scr[:, 0:W // 2, :] = jnp.zeros((NG, W // 2, 128), i32)
    vT_scr[:, 0:W] = jnp.zeros((H * 32, W), bf16)
    r = lax.broadcasted_iota(i32, (QB, QB), 0)
    c = lax.broadcasted_iota(i32, (QB, QB), 1)
    r32 = lax.broadcasted_iota(i32, (32, QB), 0)
    c32 = lax.broadcasted_iota(i32, (32, QB), 1)
    bc_scr[...] = jnp.where(r32 <= c32, 0.0, NEG).astype(f32)

    def proj_k(base, hbase, n):
        x = x_v[pl.ds(base, n), :]
        k = jnp.dot(x, wqkv_v[:, D:2 * D], preferred_element_type=f32)
        for g, s in enumerate(_slabs(k)):
            k_scr[g, pl.ds(hbase + W // 2, n // 2), :] = pltpu.bitcast(s.astype(bf16), i32)

    def proj_q(base, n):
        x = x_v[pl.ds(base, n), :]
        qT = lax.dot_general(wT_v[0:D, :], x, NT_DIMS, preferred_element_type=f32) * (DH ** -0.5 * LOG2E)
        q_scr[:, pl.ds(base, n)] = pltpu.bitcast(qT.astype(bf16), i32)

    def proj_v(base, n):
        x = x_v[pl.ds(base, n), :]
        vT = lax.dot_general(wT_v[D:2 * D, :], x, NT_DIMS, preferred_element_type=f32)
        rowi = lax.broadcasted_iota(i32, (32, n), 0)
        for hd in range(H):
            g, hh = hd // 4, hd % 4
            hm = (rowi >= 4 * hh) & (rowi < 4 * hh + DH)
            r0 = 80 * g + 16 * hh
            vT_scr[32 * hd:32 * hd + 32, pl.ds(base + W, n)] = jnp.where(hm, vT[r0:r0 + 32], 1.0).astype(bf16)

    xcopy0(0).wait()
    xcopy0(1).start()
    wcopies[0].start()
    wcopies[1].wait()
    wcopies[2].start()
    proj_k(0, 0, T0)
    xcopy0(1).wait()
    for j in range(1, NP):
        xcopy(j).start()
    for cp in wcopies[3:]:
        cp.start()
    proj_k(T0, T0 // 2, T0)
    wcopies[0].wait()
    wT_v[0:D, :] = wqkv_v[:, 0:D].astype(f32).T.astype(bf16)
    proj_q(0, TP)
    wcopies[2].wait()
    wT_v[D:2 * D, :] = wqkv_v[:, 2 * D:3 * D].astype(f32).T.astype(bf16)
    proj_v(0, TP)
    def proj_loop(j, carry):
        xcopy(j).wait()
        base = pl.multiple_of(j * TP, TP)
        proj_k(base, pl.multiple_of(j * (TP // 2), TP // 2), TP)
        proj_q(base, TP)
        proj_v(base, TP)
        return carry
    lax.fori_loop(1, NP, proj_loop, 0)

    for cp in wcopies[3:]:
        cp.wait()

    s_l = [sA, sB]
    NQ = T // QB
    lane64 = lax.broadcasted_iota(i32, (QB // 2, 128), 1)
    lane48 = lax.broadcasted_iota(i32, (48, 128), 1)
    row8 = lax.broadcasted_iota(i32, (8, QB), 0)
    col8 = lax.broadcasted_iota(i32, (8, QB), 1)

    def ocopy(i):
        st = pl.multiple_of(i * OP, OP)
        return pltpu.make_async_copy(out_v.at[pl.ds(st, OP), :], out_hbm.at[pl.ds(st, OP), :], sem_o.at[i])

    def body(i, carry):
        base = pl.multiple_of(i * T, T)
        z = jnp.minimum(i, 0)
        x = x_v[pl.ds(base, T), :]
        biases = []
        for jj in range(NQ):
            q0 = base + jj * QB
            ok = q0 >= 256
            ba_scr[jj] = jnp.where((r32 + 96 > c32) & ok, 0.0, NEG).astype(f32)
            for a in range(3):
                bm_scr[jj, 32 * a:32 * a + 32] = jnp.where(
                    c32 < 32 * (a + 1), jnp.where((32 * a + r32 > c32) & ok, 0.0, NEG),
                    jnp.where(32 * (a + 1) + r32 <= c32, 0.0, NEG)).astype(f32)
            biases.append(jnp.where(q0 >= 128, 0.0, NEG).astype(f32))

        def krows(g, jj, r0, n):
            st = pl.multiple_of(base // 2 + (jj * QB + r0) // 2, 8)
            return k_scr[g, pl.ds(st, n // 2), :]

        def qmask(u):
            jj, g = u // NG, u % NG
            qv = q_scr[40 * g:40 * g + 40, pl.ds(pl.multiple_of(base + jj * QB, QB), QB)]
            zero = jnp.zeros((8, QB), i32)
            qm, qc = [], [[], [], []]
            for hh in range(4):
                blocks = [zero] * 8
                for v in range(5):
                    lo, hi = max(10 * hh, 8 * v), min(10 * hh + 10, 8 * v + 8)
                    if lo >= hi:
                        continue
                    blk = qv[8 * v:8 * v + 8]
                    if hi - lo < 8:
                        blk = jnp.where((row8 >= lo - 8 * v) & (row8 < hi - 8 * v), blk, 0)
                    blocks[(5 * g + v) % 8] = blk
                qm.append(jnp.concatenate(blocks, axis=0))
                for a in range(3):
                    thr = 32 * (a + 1)
                    cb = []
                    for b in range(8):
                        a_, b_ = blocks[b], blocks[(b + 4) % 8]
                        if a_ is zero and b_ is zero:
                            cb.append(zero)
                        elif b_ is zero:
                            cb.append(jnp.where(col8 < thr, a_, 0))
                        elif a_ is zero:
                            cb.append(jnp.where(col8 >= thr, b_, 0))
                        else:
                            cb.append(jnp.where(col8 < thr, a_, b_))
                    qc[a].append(jnp.concatenate(cb, axis=0))
            return (pltpu.bitcast(jnp.concatenate(qm, axis=1), bf16),
                    [pltpu.bitcast(jnp.concatenate(qc[a], axis=1), bf16) for a in range(3)])

        def vmax8(s):
            mm = s[0:8]
            for r8 in range(1, s.shape[0] // 8):
                mm = jnp.maximum(mm, s[8 * r8:8 * r8 + 8])
            return mm

        def qk_piece(u, t, qms, mrun):
            jj, g = u // NG, u % NG
            slot = u % 2
            qm, qc = qms
            out = []
            if t == 2:
                early = krows(g, jj, 0, 96)
                late = pltpu.roll(krows(g, jj, 288, 96), 64, 1)
                o = (80 * g) % 128
                res = [[None] * 3 for _ in range(4)]
                for pr in range(2):
                    lsel = ((lane48 - (o + 40 * pr + 64)) & 127) < 40
                    lhs = jnp.where(lsel, late, early)
                    for a in range(3):
                        sT = jnp.dot(pltpu.bitcast(lhs[16 * a:16 * a + 16], bf16), qc[a][:, 256 * pr:256 * pr + 256],
                                     preferred_element_type=f32)
                        res[2 * pr][a] = sT[:, 0:QB]
                        res[2 * pr + 1][a] = sT[:, QB:2 * QB]
                for hh in range(4):
                    s = jnp.concatenate(res[hh], axis=0) + bm_scr[jj]
                    s_l[slot][z, hh, 192:288] = s
                    mm = vmax8(s)
                    out.append(mm if mrun is None else jnp.maximum(mrun[hh], mm))
                return out
            kw = pltpu.bitcast(krows(g, jj, 96 + 96 * t, 96), bf16)
            sT = jnp.dot(kw, qm, preferred_element_type=f32)
            for hh in range(4):
                s = sT[:, hh * QB:(hh + 1) * QB]
                if t == 0:
                    s = jnp.concatenate([s[0:32] + ba_scr[jj], s[32:96] + biases[jj]], axis=0)
                else:
                    s = jnp.concatenate([s[0:64] + biases[jj], s[64:96] + bc_scr[...]], axis=0)
                s_l[slot][z, hh, 96 * t:96 * t + 96] = s
                mm = vmax8(s)
                out.append(mm if mrun is None else jnp.maximum(mrun[hh], mm))
            return out

        cl = lax.broadcasted_iota(i32, (48, QB), 1)
        thr48 = (lax.broadcasted_iota(i32, (48, QB), 0) // 16 + 1) * 32
        def pv_t(u, t, ms, acc):
            jj, g = u // NG, u % NG
            slot = u % 2
            out = []
            for hh in range(4):
                hd = 4 * g + hh
                ex = lambda r0, n: pltpu.bitcast(jnp.exp2(s_l[slot][z, hh, r0:r0 + n] - ms[hh]).astype(bf16), i32)
                if t == 0:
                    pm = ex(192, 96)
                    pm_scr[slot, hh] = jnp.where(cl >= thr48, pm, 0)
                    p = jnp.concatenate([jnp.where(cl < thr48, pm, 0), ex(0, 32)], axis=0)
                elif t == 1:
                    p = ex(32, 128)
                else:
                    p = jnp.concatenate([ex(160, 32), pm_scr[slot, hh]], axis=0)
                p = pltpu.bitcast(p, bf16)
                vw = vT_scr[32 * hd:32 * hd + 32, pl.ds(pl.multiple_of(base + (jj + t) * QB, QB), QB)]
                d = jnp.dot(vw, p, preferred_element_type=f32)
                out.append(d if acc is None else acc[hh] + d)
            return out

        def finish(u, acc):
            jj, g = u // NG, u % NG
            os_ = []
            for hh in range(4):
                o = acc[hh]
                lrow = 31 if hh < 3 else 0
                l = o[lrow:lrow + 1, :]
                os_.append(o * (1.0 / l))
            o0, o1, o2, o3 = os_
            o_scr[jj, 80 * g:80 * g + 80, :] = jnp.concatenate(
                [o0[0:16], jnp.where(row8 < 4, o0[16:24], o1[0:8]), o1[8:24], o2[8:24],
                 jnp.where(row8 < 4, o2[24:32], o3[8:16]), o3[16:32]], axis=0)

        fin_max = lambda mrun: [jnp.max(m, axis=0, keepdims=True) for m in mrun]

        gl = jnp.sum(x.astype(f32) * gw_ref[...].astype(f32).reshape(1, D), axis=1, keepdims=True)
        gate = 0.5 * jnp.tanh(0.5 * gl) + 0.5
        hg = 0.5 * (1.0 - gate)

        def ffn1(r0, r1, c0, c1):
            h = jnp.dot(x[r0:r1], w1_v[:, c0:c1], preferred_element_type=f32)
            h = (h * hg[r0:r1]) * (jnp.tanh(0.5 * h) + 1.0)
            h_scr[r0:r1, c0:c1] = h.astype(bf16)

        def ffn2(n0, n1):
            b_scr[:, n0:n1] = jnp.dot(h_scr[...], w2_v[:, n0:n1], preferred_element_type=f32)
        jobs = []
        for c0 in range(0, F, F1C):
            for r0 in range(0, T, F1R):
                jobs.append(functools.partial(ffn1, r0, r0 + F1R, c0, c0 + F1C))
        jobs.append(functools.partial(ffn2, 512, D))
        NU = NQ * NG
        nj = len(jobs)
        tail_jobs = TAILJ
        spread = jobs[:nj - tail_jobs]
        per_unit = [[] for _ in range(NU)]
        for ji, jb in enumerate(spread):
            per_unit[(ji * (NU - 1)) // max(len(spread) - 1, 1) if SPREAD else NU - 1].append(jb)
        tails = jobs[nj - tail_jobs:]
        qm = qmask(0)
        mrun = None
        for t in range(3):
            mrun = qk_piece(0, t, qm, mrun)
        for u in range(NU):
            ms = fin_max(mrun)
            mrun = None
            acc = None
            if u + 1 < NU:
                qm = qmask(u + 1)
                for t in range(3):
                    mrun = qk_piece(u + 1, t, qm, mrun)
                    acc = pv_t(u, t, ms, acc)
                    if t < len(per_unit[u]):
                        per_unit[u][t]()
                for jb in per_unit[u][3:]:
                    jb()
            else:
                for jb in per_unit[u]:
                    jb()
                if len(tails) > 1:
                    tails[0]()
                for t in range(3):
                    acc = pv_t(u, t, ms, acc)
            finish(u, acc)
        for jb in tails[1 if len(tails) > 1 else 0:]:
            jb()
        accs = []
        for jj in range(NQ):
            o = (o_scr[jj].T * gate[jj * QB:(jj + 1) * QB]).astype(bf16)
            accs.append(o)
        o_all = jnp.concatenate(accs, axis=0)
        a = jnp.dot(o_all, wo_v[...], preferred_element_type=f32)
        out_v[pl.ds(base, T), 512:D] = (a[:, 512:D] + b_scr[:, 512:D]).astype(bf16)
        for pi in range(T // OP):
            rs = slice(pi * OP, (pi + 1) * OP)
            b0 = jnp.dot(h_scr[rs, :], w2_v[:, 0:512], preferred_element_type=f32)
            rbase = pl.multiple_of(base + pi * OP, OP)
            out_v[pl.ds(rbase, OP), 0:512] = (a[rs, 0:512] + b0).astype(bf16)
            ocopy(i * (T // OP) + pi).start()
        return carry
    lax.fori_loop(0, S // T, body, 0)
    for i in range(S // OP):
        ocopy(i).wait()

@functools.partial(jax.jit, static_argnames=("T", "TP", "F1C", "F1R", "TAILJ", "SPREAD", "OP"))
def pallas_gated_mix__sliding_block__dense_activation_silu__prompt_kernel(A_x, A_wqkv, A_wo, B_x, B_w1, B_w2, gate_w, T=512, TP=512, F1C=128, F1R=128, TAILJ=3, SPREAD=True, OP=512):
    x = A_x.reshape(S, D)
    gw = gate_w
    anyspec = pl.BlockSpec(memory_space=pl.ANY)
    NQ = T // QB
    out = pl.pallas_call(
        functools.partial(_kernel, TP=TP, T=T, F1C=F1C, F1R=F1R, TAILJ=TAILJ, SPREAD=SPREAD, OP=OP),
        in_specs=[anyspec] * 5 + [pl.BlockSpec(memory_space=pltpu.VMEM)],
        out_specs=anyspec,
        out_shape=jax.ShapeDtypeStruct((S, D), bf16),
        scratch_shapes=[
            pltpu.VMEM((S, D), bf16), pltpu.VMEM((D, 3 * D), bf16), pltpu.VMEM((D, D), bf16),
            pltpu.VMEM((D, F), bf16), pltpu.VMEM((F, D), bf16), pltpu.VMEM((2 * D, D), bf16),
            pltpu.VMEM((D // 2, S), i32), pltpu.VMEM((NG, (W + S) // 2, 128), i32), pltpu.VMEM((H * 32, W + S), bf16),
            pltpu.VMEM((1, 4, 288, QB), f32), pltpu.VMEM((1, 4, 288, QB), f32),
            pltpu.VMEM((NQ, 32, QB), f32), pltpu.VMEM((NQ, 96, QB), f32), pltpu.VMEM((32, QB), f32), pltpu.VMEM((2, 4, 48, QB), i32),
            pltpu.VMEM((NQ, D, QB), f32), pltpu.VMEM((T, F), bf16), pltpu.VMEM((T, D), f32), pltpu.VMEM((S, D), bf16),
            pltpu.SemaphoreType.DMA((S // TP,)), pltpu.SemaphoreType.DMA((2,)), pltpu.SemaphoreType.DMA((6,)), pltpu.SemaphoreType.DMA((S // OP,))],
        compiler_params=pltpu.CompilerParams(vmem_limit_bytes=100 * 2**20),
    )(x, A_wqkv, A_wo, B_w1, B_w2, gw)
    return out.reshape(1, S, D)
```

```python
import functools

import jax
import jax.numpy as jnp
from jax import lax
import jax.experimental.pallas as pl
import jax.experimental.pallas.tpu as pltpu

S, D, H, DH, F, W = 2048, 640, 32, 20, 1536, 256
NG = 8
QB = 128
TP = 512
T = 512
OP = 128
NQ = T // QB
LOG2E = 1.4426950408889634
NEG = -1e30
f32, bf16, i32 = jnp.float32, jnp.bfloat16, jnp.int32
NT_DIMS = (((1,), (1,)), ((), ()))


def _iota(shape, dim):
    return lax.broadcasted_iota(i32, shape, dim)


def _slabs(t):
    nat = [t[:, 128 * s:128 * (s + 1)] for s in range(5)]
    lane = _iota(nat[0].shape, 1)
    out = []
    for g in range(NG):
        s0, off = (80 * g) // 128, (80 * g) % 128
        out.append(nat[s0] if off + 80 <= 128 else jnp.where(lane >= off, nat[s0], nat[s0 + 1]))
    return out


def _kernel(x_hbm, wqkv_hbm, wo_hbm, w1_hbm, w2_hbm, gw_ref, out_hbm,
            x_v, wqkv_v, wo_v, w1_v, w2_v, wT_v, q_scr, k_scr, vT_scr, g_scr,
            sA, sB, ba_scr, bm_scr, bc_scr, pm_scr, o_scr, h_scr, b_scr, out_v,
            sem_x, sem_x0, sem_w, sem_o, *, F1C, F1R, TAILJ):
    NP = S // TP
    T0 = TP // 2

    def xcopy(j):
        return pltpu.make_async_copy(x_hbm.at[pl.ds(j * TP, TP), :], x_v.at[pl.ds(j * TP, TP), :], sem_x.at[j])

    def xcopy0(hf):
        return pltpu.make_async_copy(x_hbm.at[pl.ds(hf * T0, T0), :], x_v.at[pl.ds(hf * T0, T0), :], sem_x0.at[hf])

    def wcol(n, sem):
        return pltpu.make_async_copy(wqkv_hbm.at[:, pl.ds(n * D, D)], wqkv_v.at[:, pl.ds(n * D, D)], sem_w.at[sem])

    cp_wq, cp_wk, cp_wv = wcol(0, 0), wcol(1, 1), wcol(2, 2)
    cp_late = [pltpu.make_async_copy(w1_hbm, w1_v, sem_w.at[3]),
               pltpu.make_async_copy(w2_hbm, w2_v, sem_w.at[4]),
               pltpu.make_async_copy(wo_hbm, wo_v, sem_w.at[5])]

    def ocopy(n):
        st = pl.multiple_of(n * OP, OP)
        return pltpu.make_async_copy(out_v.at[pl.ds(st, OP), :], out_hbm.at[pl.ds(st, OP), :], sem_o.at[n])

    def proj_k(base, hbase, n):
        x = x_v[pl.ds(base, n), :]
        k = jnp.dot(x, wqkv_v[:, D:2 * D], preferred_element_type=f32)
        for g, s in enumerate(_slabs(k)):
            k_scr[g, pl.ds(hbase + W // 2, n // 2), :] = pltpu.bitcast(s.astype(bf16), i32)

    def proj_q(base, n):
        x = x_v[pl.ds(base, n), :]
        gl = jnp.sum(x.astype(f32) * gw_ref[...].astype(f32).reshape(1, D), axis=1, keepdims=True)
        g_scr[pl.ds(base, n), :] = 0.5 * jnp.tanh(0.5 * gl) + 0.5
        qT = lax.dot_general(wT_v[0:D, :], x, NT_DIMS, preferred_element_type=f32)
        qT = qT * (DH ** -0.5 * LOG2E)
        q_scr[:, pl.ds(base, n)] = pltpu.bitcast(qT.astype(bf16), i32)

    def proj_v(base, n):
        x = x_v[pl.ds(base, n), :]
        vT = lax.dot_general(wT_v[D:2 * D, :], x, NT_DIMS, preferred_element_type=f32)
        rowi = _iota((32, n), 0)
        for hd in range(H):
            g, hh = hd // 4, hd % 4
            hm = (rowi >= 4 * hh) & (rowi < 4 * hh + DH)
            r0 = 80 * g + 16 * hh
            vT_scr[32 * hd:32 * hd + 32, pl.ds(base + W, n)] = jnp.where(hm, vT[r0:r0 + 32], 1.0).astype(bf16)

    xcopy0(0).start()
    cp_wk.start()
    k_scr[:, 0:W // 2, :] = jnp.zeros((NG, W // 2, 128), i32)
    vT_scr[:, 0:W] = jnp.zeros((H * 32, W), bf16)
    r32, c32 = _iota((32, QB), 0), _iota((32, QB), 1)
    bc_scr[...] = jnp.where(r32 <= c32, 0.0, NEG).astype(f32)

    xcopy0(0).wait()
    xcopy0(1).start()
    cp_wq.start()
    cp_wk.wait()
    cp_wv.start()
    proj_k(0, 0, T0)
    xcopy0(1).wait()
    for j in range(1, NP):
        xcopy(j).start()
    for cp in cp_late:
        cp.start()
    proj_k(T0, T0 // 2, T0)
    cp_wq.wait()
    wT_v[0:D, :] = wqkv_v[:, 0:D].astype(f32).T.astype(bf16)
    proj_q(0, TP)
    cp_wv.wait()
    wT_v[D:2 * D, :] = wqkv_v[:, 2 * D:3 * D].astype(f32).T.astype(bf16)
    proj_v(0, TP)

    def proj_loop(j, carry):
        xcopy(j).wait()
        base = pl.multiple_of(j * TP, TP)
        proj_k(base, pl.multiple_of(j * (TP // 2), TP // 2), TP)
        proj_q(base, TP)
        proj_v(base, TP)
        return carry

    lax.fori_loop(1, NP, proj_loop, 0)
    for cp in cp_late:
        cp.wait()

    s_l = [sA, sB]
    lane48 = _iota((48, 128), 1)
    thr48 = (_iota((48, QB), 0) // 16 + 1) * 32
    row8, col8 = _iota((8, QB), 0), _iota((8, QB), 1)

    def fill_bias(jj, early_ok):
        ba_scr[jj] = jnp.where((r32 + 96 > c32) & early_ok, 0.0, NEG).astype(f32)
        for a in range(3):
            bm_scr[jj, 32 * a:32 * a + 32] = jnp.where(
                c32 < 32 * (a + 1),
                jnp.where((32 * a + r32 > c32) & early_ok, 0.0, NEG),
                jnp.where(32 * (a + 1) + r32 <= c32, 0.0, NEG)).astype(f32)

    def body(i, carry):
        base = pl.multiple_of(i * T, T)
        z = jnp.minimum(i, 0)

        @pl.when(i == 0)
        def _():
            for jj in range(NQ):
                fill_bias(jj, jj * QB >= W)

        @pl.when(i == 1)
        def _():
            for jj in range(W // QB):
                fill_bias(jj, True)

        mid_bias = [jnp.where(base + jj * QB >= QB, 0.0, NEG).astype(f32) for jj in range(NQ)]

        def krows(g, jj, r0, n):
            st = pl.multiple_of(base // 2 + (jj * QB + r0) // 2, 8)
            return k_scr[g, pl.ds(st, n // 2), :]

        def q_operands(u):
            jj, g = u // NG, u % NG
            qv = q_scr[40 * g:40 * g + 40, pl.ds(pl.multiple_of(base + jj * QB, QB), QB)]
            zero = jnp.zeros((8, QB), i32)
            qm, qc = [], [[], [], []]
            for hh in range(4):
                blocks = [zero] * 8
                for v in range(5):
                    lo, hi = max(10 * hh, 8 * v), min(10 * hh + 10, 8 * v + 8)
                    if lo >= hi:
                        continue
                    blk = qv[8 * v:8 * v + 8]
                    if hi - lo < 8:
                        blk = jnp.where((row8 >= lo - 8 * v) & (row8 < hi - 8 * v), blk, 0)
                    blocks[(5 * g + v) % 8] = blk
                qm.append(jnp.concatenate(blocks, axis=0))
                for a in range(3):
                    thr = 32 * (a + 1)
                    cb = []
                    for b in range(8):
                        a_, b_ = blocks[b], blocks[(b + 4) % 8]
                        if a_ is zero and b_ is zero:
                            cb.append(zero)
                        elif b_ is zero:
                            cb.append(jnp.where(col8 < thr, a_, 0))
                        elif a_ is zero:
                            cb.append(jnp.where(col8 >= thr, b_, 0))
                        else:
                            cb.append(jnp.where(col8 < thr, a_, b_))
                    qc[a].append(jnp.concatenate(cb, axis=0))
            return (pltpu.bitcast(jnp.concatenate(qm, axis=1), bf16),
                    [pltpu.bitcast(jnp.concatenate(qc[a], axis=1), bf16) for a in range(3)])

        def vmax8(s):
            mm = s[0:8]
            for r8 in range(1, s.shape[0] // 8):
                mm = jnp.maximum(mm, s[8 * r8:8 * r8 + 8])
            return mm

        def qk_piece(u, t, qops, mrun):
            jj, g = u // NG, u % NG
            s_ref = s_l[u % 2]
            qm, qc = qops
            if t < 2:
                kw = pltpu.bitcast(krows(g, jj, 96 + 96 * t, 96), bf16)
                sT = jnp.dot(kw, qm, preferred_element_type=f32)
                ss = []
                for hh in range(4):
                    s = sT[:, hh * QB:(hh + 1) * QB]
                    if t == 0:
                        s = jnp.concatenate([s[0:32] + ba_scr[jj], s[32:96] + mid_bias[jj]], axis=0)
                    else:
                        s = jnp.concatenate([s[0:64] + mid_bias[jj], s[64:96] + bc_scr[...]], axis=0)
                    ss.append(s)
            else:
                early = krows(g, jj, 0, 96)
                late = pltpu.roll(krows(g, jj, 288, 96), 64, 1)
                off = (80 * g) % 128
                res = [[None] * 3 for _ in range(4)]
                for pr in range(2):
                    lsel = ((lane48 - (off + 40 * pr + 64)) & 127) < 40
                    lhs = jnp.where(lsel, late, early)
                    for a in range(3):
                        sT = jnp.dot(pltpu.bitcast(lhs[16 * a:16 * a + 16], bf16),
                                     qc[a][:, 256 * pr:256 * pr + 256], preferred_element_type=f32)
                        res[2 * pr][a] = sT[:, 0:QB]
                        res[2 * pr + 1][a] = sT[:, QB:2 * QB]
                ss = [jnp.concatenate(res[hh], axis=0) + bm_scr[jj] for hh in range(4)]
            out = []
            for hh in range(4):
                s_ref[z, hh, 96 * t:96 * t + 96] = ss[hh]
                mm = vmax8(ss[hh])
                out.append(mm if mrun is None else jnp.maximum(mrun[hh], mm))
            return out

        def pv_piece(u, t, ms, acc):
            jj, g = u // NG, u % NG
            slot = u % 2
            s_ref = s_l[slot]
            out = []
            for hh in range(4):
                hd = 4 * g + hh

                def ex(r0, n):
                    return pltpu.bitcast(jnp.exp2(s_ref[z, hh, r0:r0 + n] - ms[hh]).astype(bf16), i32)

                if t == 0:
                    pm = ex(192, 96)
                    pm_scr[slot, hh] = jnp.where(lane48 >= thr48, pm, 0)
                    p = jnp.concatenate([jnp.where(lane48 < thr48, pm, 0), ex(0, 32)], axis=0)
                elif t == 1:
                    p = ex(32, 128)
                else:
                    p = jnp.concatenate([ex(160, 32), pm_scr[slot, hh]], axis=0)
                vw = vT_scr[32 * hd:32 * hd + 32, pl.ds(pl.multiple_of(base + (jj + t) * QB, QB), QB)]
                d = jnp.dot(vw, pltpu.bitcast(p, bf16), preferred_element_type=f32)
                out.append(d if acc is None else acc[hh] + d)
            return out

        def finish(u, acc):
            jj, g = u // NG, u % NG
            os_ = []
            for hh in range(4):
                lrow = 31 if hh < 3 else 0
                os_.append(acc[hh] * (1.0 / acc[hh][lrow:lrow + 1, :]))
            o0, o1, o2, o3 = os_
            o_scr[jj, 80 * g:80 * g + 80, :] = jnp.concatenate(
                [o0[0:16], jnp.where(row8 < 4, o0[16:24], o1[0:8]), o1[8:24],
                 o2[8:24], jnp.where(row8 < 4, o2[24:32], o3[8:16]), o3[16:32]], axis=0)

        x = x_v[pl.ds(base, T), :]
        gate = g_scr[pl.ds(base, T), :]
        hg = 0.5 * (1.0 - gate)

        def ffn1(r0, c0):
            h = jnp.dot(x[r0:r0 + F1R], w1_v[:, c0:c0 + F1C], preferred_element_type=f32)
            h = (h * hg[r0:r0 + F1R]) * (jnp.tanh(0.5 * h) + 1.0)
            h_scr[r0:r0 + F1R, c0:c0 + F1C] = h.astype(bf16)

        def ffn2_tail():
            b_scr[...] = jnp.dot(h_scr[...], w2_v[:, 512:D], preferred_element_type=f32)

        jobs = [functools.partial(ffn1, r0, c0) for c0 in range(0, F, F1C) for r0 in range(0, T, F1R)]
        jobs.append(ffn2_tail)
        NU = NQ * NG
        spread, tails = jobs[:len(jobs) - TAILJ], jobs[len(jobs) - TAILJ:]
        per_unit = [[] for _ in range(NU)]
        for ji, jb in enumerate(spread):
            per_unit[(ji * (NU - 1)) // (len(spread) - 1)].append(jb)

        qops = q_operands(0)
        mrun = None
        for t in range(3):
            mrun = qk_piece(0, t, qops, mrun)
        for u in range(NU):
            ms = [jnp.max(m, axis=0, keepdims=True) for m in mrun]
            mrun, acc = None, None
            if u + 1 < NU:
                qops = q_operands(u + 1)
                for t in range(3):
                    mrun = qk_piece(u + 1, t, qops, mrun)
                    acc = pv_piece(u, t, ms, acc)
                    if t < len(per_unit[u]):
                        per_unit[u][t]()
                for jb in per_unit[u][3:]:
                    jb()
            else:
                for jb in per_unit[u]:
                    jb()
                tails[0]()
                for t in range(3):
                    acc = pv_piece(u, t, ms, acc)
            finish(u, acc)
        for jb in tails[1:]:
            jb()

        o_all = jnp.concatenate(
            [(o_scr[jj].T * gate[jj * QB:(jj + 1) * QB]).astype(bf16) for jj in range(NQ)], axis=0)
        a = jnp.dot(o_all, wo_v[...], preferred_element_type=f32)
        out_v[pl.ds(base, T), 512:D] = (a[:, 512:D] + b_scr[...]).astype(bf16)
        b0 = jnp.dot(h_scr[...], w2_v[:, 0:512], preferred_element_type=f32)
        for pi in range(T // OP):
            rs = slice(pi * OP, (pi + 1) * OP)
            out_v[pl.ds(pl.multiple_of(base + pi * OP, OP), OP), 0:512] = (a[rs, 0:512] + b0[rs]).astype(bf16)
            ocopy(i * (T // OP) + pi).start()
        return carry

    lax.fori_loop(0, S // T, body, 0)
    for n in range(S // OP):
        ocopy(n).wait()


@functools.partial(jax.jit, static_argnames=("F1C", "F1R", "TAILJ"))
def pallas_gated_mix__sliding_block__dense_activation_silu__prompt_kernel(
        A_x, A_wqkv, A_wo, B_x, B_w1, B_w2, gate_w, F1C=128, F1R=128, TAILJ=3):
    del B_x
    hbm = pl.BlockSpec(memory_space=pl.ANY)
    out = pl.pallas_call(
        functools.partial(_kernel, F1C=F1C, F1R=F1R, TAILJ=TAILJ),
        in_specs=[hbm] * 5 + [pl.BlockSpec(memory_space=pltpu.VMEM)],
        out_specs=hbm,
        out_shape=jax.ShapeDtypeStruct((S, D), bf16),
        scratch_shapes=[
            pltpu.VMEM((S, D), bf16),
            pltpu.VMEM((D, 3 * D), bf16),
            pltpu.VMEM((D, D), bf16),
            pltpu.VMEM((D, F), bf16),
            pltpu.VMEM((F, D), bf16),
            pltpu.VMEM((2 * D, D), bf16),
            pltpu.VMEM((D // 2, S), i32),
            pltpu.VMEM((NG, (W + S) // 2, 128), i32),
            pltpu.VMEM((H * 32, W + S), bf16),
            pltpu.VMEM((S, 1), f32),
            pltpu.VMEM((1, 4, 288, QB), f32),
            pltpu.VMEM((1, 4, 288, QB), f32),
            pltpu.VMEM((NQ, 32, QB), f32),
            pltpu.VMEM((NQ, 96, QB), f32),
            pltpu.VMEM((32, QB), f32),
            pltpu.VMEM((2, 4, 48, QB), i32),
            pltpu.VMEM((NQ, D, QB), f32),
            pltpu.VMEM((T, F), bf16),
            pltpu.VMEM((T, D - 512), f32),
            pltpu.VMEM((S, D), bf16),
            pltpu.SemaphoreType.DMA((S // TP,)),
            pltpu.SemaphoreType.DMA((2,)),
            pltpu.SemaphoreType.DMA((6,)),
            pltpu.SemaphoreType.DMA((S // OP,)),
        ],
        compiler_params=pltpu.CompilerParams(vmem_limit_bytes=100 * 2**20),
    )(A_x.reshape(S, D), A_wqkv, A_wo, B_w1, B_w2, gate_w)
    return out.reshape(1, S, D)
```

```python
import functools

import jax
import jax.numpy as jnp
from jax import lax
import jax.experimental.pallas as pl
import jax.experimental.pallas.tpu as pltpu

S, D, H, DH, F, W = 2048, 640, 32, 20, 1536, 256
NG = 8
QB = 128
TP = 512
T = 512
OP = 128
NQ = T // QB
F1C, F1R = 128, 128
PRE, TAILJ = 3, 3
LOG2E = 1.4426950408889634
NEG = -1e30
f32, bf16, i32 = jnp.float32, jnp.bfloat16, jnp.int32
NT_DIMS = (((1,), (1,)), ((), ()))


def _iota(shape, dim):
    return lax.broadcasted_iota(i32, shape, dim)


def _slabs(t):
    nat = [t[:, 128 * s:128 * (s + 1)] for s in range(5)]
    lane = _iota(nat[0].shape, 1)
    out = []
    for g in range(NG):
        s0, off = (80 * g) // 128, (80 * g) % 128
        out.append(nat[s0] if off + 80 <= 128 else jnp.where(lane >= off, nat[s0], nat[s0 + 1]))
    return out


def _kernel(x_hbm, wqkv_hbm, wo_hbm, w1_hbm, w2_hbm, gw_ref, out_hbm,
            x_v, wqkv_v, wo_v, w1_v, w2_v, wT_v, q_scr, k_scr, vT_scr, g_scr,
            sA, sB, ba_scr, bm_scr, bc_scr, pm_scr, o_scr, h_scr, b_scr, out_v,
            sem_x, sem_x0, sem_w, sem_o):
    NP = S // TP
    T0 = TP // 2

    def xcopy(j):
        return pltpu.make_async_copy(x_hbm.at[pl.ds(j * TP, TP), :], x_v.at[pl.ds(j * TP, TP), :], sem_x.at[j])

    def xcopy0(hf):
        return pltpu.make_async_copy(x_hbm.at[pl.ds(hf * T0, T0), :], x_v.at[pl.ds(hf * T0, T0), :], sem_x0.at[hf])

    def wcol(n, sem):
        return pltpu.make_async_copy(wqkv_hbm.at[:, pl.ds(n * D, D)], wqkv_v.at[:, pl.ds(n * D, D)], sem_w.at[sem])

    cp_wq, cp_wk, cp_wv = wcol(0, 0), wcol(1, 1), wcol(2, 2)
    cp_late = [pltpu.make_async_copy(w1_hbm, w1_v, sem_w.at[3]),
               pltpu.make_async_copy(w2_hbm, w2_v, sem_w.at[4]),
               pltpu.make_async_copy(wo_hbm, wo_v, sem_w.at[5])]

    def ocopy(n):
        st = pl.multiple_of(n * OP, OP)
        return pltpu.make_async_copy(out_v.at[pl.ds(st, OP), :], out_hbm.at[pl.ds(st, OP), :], sem_o.at[n])

    def proj_k(base, hbase, n):
        x = x_v[pl.ds(base, n), :]
        k = jnp.dot(x, wqkv_v[:, D:2 * D], preferred_element_type=f32)
        for g, s in enumerate(_slabs(k)):
            k_scr[g, pl.ds(hbase + W // 2, n // 2), :] = pltpu.bitcast(s.astype(bf16), i32)

    def proj_q(base, n):
        x = x_v[pl.ds(base, n), :]
        gl = jnp.sum(x.astype(f32) * gw_ref[...].astype(f32).reshape(1, D), axis=1, keepdims=True)
        g_scr[pl.ds(base, n), :] = 0.5 * jnp.tanh(0.5 * gl) + 0.5
        qT = lax.dot_general(wT_v[0:D, :], x, NT_DIMS, preferred_element_type=f32)
        qT = qT * (DH ** -0.5 * LOG2E)
        q_scr[:, pl.ds(base, n)] = pltpu.bitcast(qT.astype(bf16), i32)

    def proj_v(base, n):
        x = x_v[pl.ds(base, n), :]
        vT = lax.dot_general(wT_v[D:2 * D, :], x, NT_DIMS, preferred_element_type=f32)
        rowi = _iota((32, n), 0)
        for hd in range(H):
            g, hh = hd // 4, hd % 4
            hm = (rowi >= 4 * hh) & (rowi < 4 * hh + DH)
            r0 = 80 * g + 16 * hh
            vT_scr[32 * hd:32 * hd + 32, pl.ds(base + W, n)] = jnp.where(hm, vT[r0:r0 + 32], 1.0).astype(bf16)

    xcopy0(0).start()
    cp_wk.start()
    k_scr[:, 0:W // 2, :] = jnp.zeros((NG, W // 2, 128), i32)
    vT_scr[:, 0:W] = jnp.zeros((H * 32, W), bf16)
    r32, c32 = _iota((32, QB), 0), _iota((32, QB), 1)
    bc_scr[...] = jnp.where(r32 <= c32, 0.0, NEG).astype(f32)

    xcopy0(0).wait()
    xcopy0(1).start()
    cp_wq.start()
    cp_wk.wait()
    cp_wv.start()
    proj_k(0, 0, T0)
    xcopy0(1).wait()
    for j in range(1, NP):
        xcopy(j).start()
    for cp in cp_late:
        cp.start()
    proj_k(T0, T0 // 2, T0)
    cp_wq.wait()
    wT_v[0:D, :] = wqkv_v[:, 0:D].astype(f32).T.astype(bf16)
    proj_q(0, TP)
    cp_wv.wait()
    wT_v[D:2 * D, :] = wqkv_v[:, 2 * D:3 * D].astype(f32).T.astype(bf16)
    proj_v(0, TP)

    def proj_loop(j, carry):
        xcopy(j).wait()
        base = pl.multiple_of(j * TP, TP)
        proj_k(base, pl.multiple_of(j * (TP // 2), TP // 2), TP)
        proj_q(base, TP)
        proj_v(base, TP)
        return carry

    lax.fori_loop(1, NP, proj_loop, 0)
    for cp in cp_late:
        cp.wait()

    s_l = [sA, sB]
    lane48 = _iota((48, 128), 1)
    thr48 = (_iota((48, QB), 0) // 16 + 1) * 32
    row8, col8 = _iota((8, QB), 0), _iota((8, QB), 1)

    def fill_bias(jj, early_ok):
        ba_scr[jj] = jnp.where((r32 + 96 > c32) & early_ok, 0.0, NEG).astype(f32)
        for a in range(3):
            bm_scr[jj, 32 * a:32 * a + 32] = jnp.where(
                c32 < 32 * (a + 1),
                jnp.where((32 * a + r32 > c32) & early_ok, 0.0, NEG),
                jnp.where(32 * (a + 1) + r32 <= c32, 0.0, NEG)).astype(f32)

    def body(i, carry):
        base = pl.multiple_of(i * T, T)
        z = jnp.minimum(i, 0)

        @pl.when(i == 0)
        def _():
            for jj in range(NQ):
                fill_bias(jj, jj * QB >= W)

        @pl.when(i == 1)
        def _():
            for jj in range(W // QB):
                fill_bias(jj, True)

        mid_bias = [jnp.where(base + jj * QB >= QB, 0.0, NEG).astype(f32) for jj in range(NQ)]

        def krows(g, jj, r0, n):
            st = pl.multiple_of(base // 2 + (jj * QB + r0) // 2, 8)
            return k_scr[g, pl.ds(st, n // 2), :]

        def q_operands(u):
            jj, g = u // NG, u % NG
            qv = q_scr[40 * g:40 * g + 40, pl.ds(pl.multiple_of(base + jj * QB, QB), QB)]
            zero = jnp.zeros((8, QB), i32)
            qm, qc = [], [[], [], []]
            for hh in range(4):
                blocks = [zero] * 8
                for v in range(5):
                    lo, hi = max(10 * hh, 8 * v), min(10 * hh + 10, 8 * v + 8)
                    if lo >= hi:
                        continue
                    blk = qv[8 * v:8 * v + 8]
                    if hi - lo < 8:
                        blk = jnp.where((row8 >= lo - 8 * v) & (row8 < hi - 8 * v), blk, 0)
                    blocks[(5 * g + v) % 8] = blk
                qm.append(jnp.concatenate(blocks, axis=0))
                for a in range(3):
                    thr = 32 * (a + 1)
                    cb = []
                    for b in range(8):
                        a_, b_ = blocks[b], blocks[(b + 4) % 8]
                        if a_ is zero and b_ is zero:
                            cb.append(zero)
                        elif b_ is zero:
                            cb.append(jnp.where(col8 < thr, a_, 0))
                        elif a_ is zero:
                            cb.append(jnp.where(col8 >= thr, b_, 0))
                        else:
                            cb.append(jnp.where(col8 < thr, a_, b_))
                    qc[a].append(jnp.concatenate(cb, axis=0))
            return (pltpu.bitcast(jnp.concatenate(qm, axis=1), bf16),
                    [pltpu.bitcast(jnp.concatenate(qc[a], axis=1), bf16) for a in range(3)])

        def vmax8(s):
            mm = s[0:8]
            for r8 in range(1, s.shape[0] // 8):
                mm = jnp.maximum(mm, s[8 * r8:8 * r8 + 8])
            return mm

        def qk_piece(u, t, qops, mrun):
            jj, g = u // NG, u % NG
            s_ref = s_l[u % 2]
            qm, qc = qops
            if t < 2:
                kw = pltpu.bitcast(krows(g, jj, 96 + 96 * t, 96), bf16)
                sT = jnp.dot(kw, qm, preferred_element_type=f32)
                ss = []
                for hh in range(4):
                    s = sT[:, hh * QB:(hh + 1) * QB]
                    if t == 0:
                        s = jnp.concatenate([s[0:32] + ba_scr[jj], s[32:96] + mid_bias[jj]], axis=0)
                    else:
                        s = jnp.concatenate([s[0:64] + mid_bias[jj], s[64:96] + bc_scr[...]], axis=0)
                    ss.append(s)
            else:
                early = krows(g, jj, 0, 96)
                late = pltpu.roll(krows(g, jj, 288, 96), 64, 1)
                off = (80 * g) % 128
                res = [[None] * 3 for _ in range(4)]
                for pr in range(2):
                    lsel = ((lane48 - (off + 40 * pr + 64)) & 127) < 40
                    lhs = jnp.where(lsel, late, early)
                    for a in range(3):
                        sT = jnp.dot(pltpu.bitcast(lhs[16 * a:16 * a + 16], bf16),
                                     qc[a][:, 256 * pr:256 * pr + 256], preferred_element_type=f32)
                        res[2 * pr][a] = sT[:, 0:QB]
                        res[2 * pr + 1][a] = sT[:, QB:2 * QB]
                ss = [jnp.concatenate(res[hh], axis=0) + bm_scr[jj] for hh in range(4)]
            out = []
            for hh in range(4):
                s_ref[z, hh, 96 * t:96 * t + 96] = ss[hh]
                mm = vmax8(ss[hh])
                out.append(mm if mrun is None else jnp.maximum(mrun[hh], mm))
            return out

        def pv_piece(u, t, ms, acc):
            jj, g = u // NG, u % NG
            slot = u % 2
            s_ref = s_l[slot]
            out = []
            for hh in range(4):
                hd = 4 * g + hh

                def ex(r0, n):
                    return pltpu.bitcast(jnp.exp2(s_ref[z, hh, r0:r0 + n] - ms[hh]).astype(bf16), i32)

                if t == 0:
                    pm = ex(192, 96)
                    pm_scr[slot, hh] = jnp.where(lane48 >= thr48, pm, 0)
                    p = jnp.concatenate([jnp.where(lane48 < thr48, pm, 0), ex(0, 32)], axis=0)
                elif t == 1:
                    p = ex(32, 128)
                else:
                    p = jnp.concatenate([ex(160, 32), pm_scr[slot, hh]], axis=0)
                vw = vT_scr[32 * hd:32 * hd + 32, pl.ds(pl.multiple_of(base + (jj + t) * QB, QB), QB)]
                d = jnp.dot(vw, pltpu.bitcast(p, bf16), preferred_element_type=f32)
                out.append(d if acc is None else acc[hh] + d)
            return out

        def finish(u, acc):
            jj, g = u // NG, u % NG
            os_ = []
            for hh in range(4):
                lrow = 31 if hh < 3 else 0
                os_.append(acc[hh] * (1.0 / acc[hh][lrow:lrow + 1, :]))
            o0, o1, o2, o3 = os_
            o_scr[jj, 80 * g:80 * g + 80, :] = jnp.concatenate(
                [o0[0:16], jnp.where(row8 < 4, o0[16:24], o1[0:8]), o1[8:24],
                 o2[8:24], jnp.where(row8 < 4, o2[24:32], o3[8:16]), o3[16:32]], axis=0)

        x = x_v[pl.ds(base, T), :]
        gate = g_scr[pl.ds(base, T), :]
        hg = 0.5 * (1.0 - gate)

        def ffn1(r0, c0):
            h = jnp.dot(x[r0:r0 + F1R], w1_v[:, c0:c0 + F1C], preferred_element_type=f32)
            h = (h * hg[r0:r0 + F1R]) * (jnp.tanh(0.5 * h) + 1.0)
            h_scr[r0:r0 + F1R, c0:c0 + F1C] = h.astype(bf16)

        def ffn2_tail():
            b_scr[...] = jnp.dot(h_scr[...], w2_v[:, 512:D], preferred_element_type=f32)

        jobs = [functools.partial(ffn1, r0, c0) for c0 in range(0, F, F1C) for r0 in range(0, T, F1R)]
        jobs.append(ffn2_tail)
        NU = NQ * NG
        pre, spread, tails = jobs[:PRE], jobs[PRE:len(jobs) - TAILJ], jobs[len(jobs) - TAILJ:]
        per_unit = [[] for _ in range(NU)]
        for ji, jb in enumerate(spread):
            per_unit[(ji * (NU - 1)) // (len(spread) - 1)].append(jb)

        qops = q_operands(0)
        mrun = None
        for t in range(3):
            mrun = qk_piece(0, t, qops, mrun)
        for jb in pre:
            jb()
        for u in range(NU):
            ms = [jnp.max(m, axis=0, keepdims=True) for m in mrun]
            mrun, acc = None, None
            if u + 1 < NU:
                qops = q_operands(u + 1)
                for t in range(3):
                    mrun = qk_piece(u + 1, t, qops, mrun)
                    acc = pv_piece(u, t, ms, acc)
                    if t < len(per_unit[u]):
                        per_unit[u][t]()
                for jb in per_unit[u][3:]:
                    jb()
            else:
                for jb in per_unit[u]:
                    jb()
                tails[0]()
                for t in range(3):
                    acc = pv_piece(u, t, ms, acc)
            finish(u, acc)
        for jb in tails[1:]:
            jb()

        o_all = jnp.concatenate(
            [(o_scr[jj].T * gate[jj * QB:(jj + 1) * QB]).astype(bf16) for jj in range(NQ)], axis=0)
        a = jnp.dot(o_all, wo_v[...], preferred_element_type=f32)
        out_v[pl.ds(base, T), 512:D] = (a[:, 512:D] + b_scr[...]).astype(bf16)
        b0 = jnp.dot(h_scr[...], w2_v[:, 0:512], preferred_element_type=f32)
        for pi in range(T // OP):
            rs = slice(pi * OP, (pi + 1) * OP)
            out_v[pl.ds(pl.multiple_of(base + pi * OP, OP), OP), 0:512] = (a[rs, 0:512] + b0[rs]).astype(bf16)
            ocopy(i * (T // OP) + pi).start()
        return carry

    lax.fori_loop(0, S // T, body, 0)
    for n in range(S // OP):
        ocopy(n).wait()


@jax.jit
def pallas_gated_mix__sliding_block__dense_activation_silu__prompt_kernel(
        A_x, A_wqkv, A_wo, B_x, B_w1, B_w2, gate_w):
    del B_x
    hbm = pl.BlockSpec(memory_space=pl.ANY)
    out = pl.pallas_call(
        _kernel,
        in_specs=[hbm] * 5 + [pl.BlockSpec(memory_space=pltpu.VMEM)],
        out_specs=hbm,
        out_shape=jax.ShapeDtypeStruct((S, D), bf16),
        scratch_shapes=[
            pltpu.VMEM((S, D), bf16),
            pltpu.VMEM((D, 3 * D), bf16),
            pltpu.VMEM((D, D), bf16),
            pltpu.VMEM((D, F), bf16),
            pltpu.VMEM((F, D), bf16),
            pltpu.VMEM((2 * D, D), bf16),
            pltpu.VMEM((D // 2, S), i32),
            pltpu.VMEM((NG, (W + S) // 2, 128), i32),
            pltpu.VMEM((H * 32, W + S), bf16),
            pltpu.VMEM((S, 1), f32),
            pltpu.VMEM((1, 4, 288, QB), f32),
            pltpu.VMEM((1, 4, 288, QB), f32),
            pltpu.VMEM((NQ, 32, QB), f32),
            pltpu.VMEM((NQ, 96, QB), f32),
            pltpu.VMEM((32, QB), f32),
            pltpu.VMEM((2, 4, 48, QB), i32),
            pltpu.VMEM((NQ, D, QB), f32),
            pltpu.VMEM((T, F), bf16),
            pltpu.VMEM((T, D - 512), f32),
            pltpu.VMEM((S, D), bf16),
            pltpu.SemaphoreType.DMA((S // TP,)),
            pltpu.SemaphoreType.DMA((2,)),
            pltpu.SemaphoreType.DMA((6,)),
            pltpu.SemaphoreType.DMA((S // OP,)),
        ],
        compiler_params=pltpu.CompilerParams(vmem_limit_bytes=100 * 2**20),
    )(A_x.reshape(S, D), A_wqkv, A_wo, B_w1, B_w2, gate_w)
    return out.reshape(1, S, D)
```
